```python
import os as _os
_os.environ.setdefault("JAX_PLATFORMS", "cpu")
import jax
import jax.numpy as jnp

def _softmax(x, axis=-1):
    return jax.nn.softmax(x, axis=axis)
def _gelu(x):
    return jax.nn.gelu(x, approximate=True)
def _silu(x):
    return jax.nn.silu(x)
def _sigmoid(x):
    return jax.nn.sigmoid(x)
def _layernorm(x, axis=-1, eps=1e-5):
    m = jnp.mean(x, axis=axis, keepdims=True)
    v = jnp.var(x, axis=axis, keepdims=True)
    return (x - m) / jnp.sqrt(v + eps)
def _scatter_add(tgt, idx, src, axis=0):
    return tgt.at[idx].add(src)
def _segment_sum(src, seg, n):
    return jax.ops.segment_sum(src, seg, n)
class _Rng:
    def __init__(self, key):
        self._k = key
    def _next(self):
        self._k, sub = jax.random.split(self._k)
        return sub
    def normal(self, shape):
        return jax.random.normal(self._next(), shape, dtype=jnp.bfloat16)
    def randint(self, lo, hi, shape):
        return jax.random.randint(self._next(), shape, lo, hi, dtype=jnp.int32)
    def uniform(self, shape, lo=0.0, hi=1.0):
        return jax.random.uniform(self._next(), shape, jnp.bfloat16, lo, hi)
    def permutation(self, n):
        return jax.random.permutation(self._next(), n)


kernel_name = 'sequential_preLN__linear_attn_block__dense_activation_squared_relu__prompt'

def setup_inputs():
    _rng = _Rng(jax.random.key(int.from_bytes(__import__("os").urandom(4), "little")))
    _w = (lambda a: (lambda t: t.astype(jnp.bfloat16) if jnp.issubdtype(t.dtype, jnp.floating) else t)(jnp.asarray(a)))
    def _A_setup():
        B, S, D = 1, 2048, 576
        return {
            "x": _w((lambda *s: _rng.normal(s) * 0.05)(B, S, D)),
            "wqkv": _w((lambda *s: _rng.normal(s) * 0.1)(D, 3 * D)),
            "wo": _w((lambda *s: _rng.normal(s) * 0.05)(D, D)),
        }
    _A_in = _A_setup()

    def _B_setup():
        B, S, D, F = 1, 2048, 576, 4608
        return {
            "x": _w((lambda *s: _rng.normal(s) * 0.05)(B, S, D)),
            "w1": _w((lambda *s: _rng.normal(s) * 0.05)(D, F)),
            "b1": _w((lambda *s: _rng.normal(s) * 0.05)(F)),
            "w2": _w((lambda *s: _rng.normal(s) * 0.05)(F, D)),
            "b2": _w((lambda *s: _rng.normal(s) * 0.05)(D)),
        }
    _B_in = _B_setup()

    return {
        "A_x": _A_in["x"],
        "A_wqkv": _A_in["wqkv"],
        "A_wo": _A_in["wo"],
        "B_x": _B_in["x"],
        "B_w1": _B_in["w1"],
        "B_b1": _B_in["b1"],
        "B_w2": _B_in["w2"],
        "B_b2": _B_in["b2"],
    }

def reference(A_x, A_wqkv, A_wo, B_x, B_w1, B_b1, B_w2, B_b2):
    def _A_ref(x, wqkv, wo):
        B, S, D = x.shape
        H = 32; Dh = D // H
        qkv = (lambda x, *d: x.transpose(*d))((x @ wqkv).reshape(B, S, 3, H, Dh), 2, 0, 3, 1, 4)
        q, k, v = qkv[0], qkv[1], qkv[2]
        phi = lambda t: jnp.where(t > 0, t + 1, jnp.exp(t)) + 1e-6
        pq, pk = phi(q), phi(k)
        kv = jnp.einsum("bhsd,bhse->bhde", pk, v)
        z = jnp.einsum("bhsd->bhd", pk)
        num = jnp.einsum("bhqd,bhde->bhqe", pq, kv)
        den = jnp.einsum("bhqd,bhd->bhq", pq, z)[..., None] + 1e-6
        o = num / den
        return (lambda x, *d: x.transpose(*d))(o, 0, 2, 1, 3).reshape(B, S, D) @ wo

    def _B_ref(x, w1, b1, w2, b2):
        h = jnp.einsum("bsd,df->bsf", x, w1) + b1
        zero = jnp.zeros_like(h)
        r = jnp.where(h > zero, h, zero)
        h = r * r
        out = jnp.einsum("bsf,fd->bsd", h, w2) + b2
        return out

    x = A_x
    h = x + _A_ref(_layernorm(x, axis=-1), A_wqkv, A_wo)
    h2 = h + _B_ref(_layernorm(h, axis=-1), B_w1, B_b1, B_w2, B_b2)
    return h2
```

```python
import functools

import jax
import jax.numpy as jnp
from jax import lax
import jax.experimental.pallas as pl
import jax.experimental.pallas.tpu as pltpu

H = 32
LN_EPS = 1e-5
PHI_EPS = 1e-6
DEN_EPS = 1e-6

TM = 512
TF = 512

NT_DIMS = (((1,), (1,)), ((), ()))


def _ln_t(x):
    m = jnp.mean(x, axis=0, keepdims=True)
    xc = x - m
    v = jnp.mean(xc * xc, axis=0, keepdims=True)
    return xc * lax.rsqrt(v + LN_EPS)


def _phi(t):
    return jnp.where(t > 0, t + 1.0, jnp.exp(t)) + PHI_EPS


def _kernel(x_ref, wqkv_hbm, wo_hbm, w1_hbm, b1_ref, w2t_hbm, b2_ref, o_ref,
            wqkv_s, wo_s, w1_s, w2t_s, wqkvt_s, pqt_s, kvt_s, mt_s, zc_s, et_s,
            b1_s, b2_s, sems, *, S, D, F, nt):
    f32 = jnp.float32
    bf16 = jnp.bfloat16
    DH = D // H
    step = pl.program_id(0)

    def wcopy(src, dst, i):
        return pltpu.make_async_copy(src, dst, sems.at[i])

    @pl.when(step == 0)
    def _init():
        c = wcopy(wqkv_hbm, wqkv_s, 0)
        c.start()
        c.wait()
        wcopy(wo_hbm, wo_s, 1).start()
        wcopy(w1_hbm, w1_s, 2).start()
        wcopy(w2t_hbm, w2t_s, 3).start()
        wqkvt_s[...] = jnp.transpose(wqkv_s[...].astype(f32)).astype(bf16)
        kvt_s[...] = jnp.zeros(kvt_s.shape, f32)

    @pl.when(step < nt)
    def _phase1():
        x = x_ref[...].astype(f32)
        ln = _ln_t(x).astype(bf16)
        qkv = jnp.dot(wqkvt_s[...], ln, preferred_element_type=f32)
        col0 = pl.multiple_of(step * TM, TM)
        pqt_s[:, pl.ds(col0, TM)] = _phi(qkv[0:D]).astype(bf16)
        pk = _phi(qkv[D:2 * D]).astype(bf16)
        ones_rows = jnp.where(
            lax.broadcasted_iota(jnp.int32, (16, TM), 0) == 0, 1.0, 0.0).astype(bf16)
        v_aug = jnp.concatenate([qkv[2 * D:3 * D].astype(bf16), ones_rows], axis=0)
        kvt_s[...] += lax.dot_general(v_aug, pk, NT_DIMS, preferred_element_type=f32)

    @pl.when(step == nt)
    def _mid():
        wcopy(wo_hbm, wo_s, 1).wait()
        r = lax.broadcasted_iota(jnp.int32, (D, D), 0) // DH
        c = lax.broadcasted_iota(jnp.int32, (D, D), 1) // DH
        kvtbd = jnp.where(r == c, kvt_s[0:D, :], 0.0).astype(bf16)
        wot = jnp.transpose(wo_s[...].astype(f32)).astype(bf16)
        mt_s[...] = jnp.dot(wot, kvtbd, preferred_element_type=f32).astype(bf16)
        z = kvt_s[D:D + 1, :]
        rr = lax.broadcasted_iota(jnp.int32, (2 * H, D), 0)
        cc = lax.broadcasted_iota(jnp.int32, (2 * H, D), 1) // DH
        zc_s[...] = jnp.where((rr % H) == cc, z, 0.0).astype(bf16)
        er = lax.broadcasted_iota(jnp.int32, (D, 2 * H), 0) // DH
        ec = lax.broadcasted_iota(jnp.int32, (D, 2 * H), 1)
        et_s[...] = jnp.where((ec % H) == er, 1.0, 0.0).astype(bf16)
        b1_s[...] = b1_ref[...].astype(f32).reshape(1, F)
        b2row = jnp.broadcast_to(b2_ref[...].astype(f32).reshape(1, D), (128, D))
        b2_s[...] = jnp.transpose(b2row)
        wcopy(w1_hbm, w1_s, 2).wait()
        wcopy(w2t_hbm, w2t_s, 3).wait()

    @pl.when(step >= nt)
    def _phase2():
        col0 = pl.multiple_of((step - nt) * TM, TM)
        pq = pqt_s[:, pl.ds(col0, TM)]
        den = jnp.dot(zc_s[...], pq, preferred_element_type=f32)
        rcp = 1.0 / (den + DEN_EPS)
        r_hi = rcp.astype(bf16)
        r_lo = (rcp - r_hi.astype(f32)).astype(bf16)
        row = lax.broadcasted_iota(jnp.int32, (2 * H, TM), 0)
        rr = jnp.where(row < H, r_hi, r_lo)
        rexp = jnp.dot(et_s[...], rr, preferred_element_type=f32)
        pqs = (pq.astype(f32) * rexp).astype(bf16)
        attn = jnp.dot(mt_s[...], pqs, preferred_element_type=f32)
        h = x_ref[...].astype(f32) + attn
        ln2 = jnp.transpose(_ln_t(h)).astype(bf16)
        acc = h + jnp.concatenate([b2_s[...]] * (TM // 128), axis=1)
        for j in range(F // TF):
            a = jnp.dot(ln2, w1_s[:, j * TF:(j + 1) * TF],
                        preferred_element_type=f32)
            a = a + b1_s[:, j * TF:(j + 1) * TF]
            a = jnp.maximum(a, 0.0)
            a = (a * a).astype(bf16)
            acc = acc + lax.dot_general(w2t_s[:, j * TF:(j + 1) * TF], a, NT_DIMS,
                                        preferred_element_type=f32)
        o_ref[...] = acc.astype(o_ref.dtype)


@jax.jit
def pallas_sequential_preLN__linear_attn_block__dense_activation_squared_relu__prompt_kernel(
    A_x: jax.Array,
    A_wqkv: jax.Array,
    A_wo: jax.Array,
    B_x: jax.Array,
    B_w1: jax.Array,
    B_b1: jax.Array,
    B_w2: jax.Array,
    B_b2: jax.Array,
):
    del B_x
    B, S, D = A_x.shape
    F = B_w1.shape[1]
    assert B == 1 and S % TM == 0 and F % TF == 0 and D % H == 0
    nt = S // TM
    bf16 = jnp.bfloat16
    f32 = jnp.float32

    kern = functools.partial(_kernel, S=S, D=D, F=F, nt=nt)
    hbm_spec = pl.BlockSpec(memory_space=pltpu.HBM)
    xt = jnp.transpose(A_x, (0, 2, 1))
    w2t = jnp.transpose(B_w2, (1, 0))
    out_t = pl.pallas_call(
        kern,
        grid=(2 * nt,),
        in_specs=[
            pl.BlockSpec((None, D, TM), lambda s: (0, 0, s % nt)),
            hbm_spec,
            hbm_spec,
            hbm_spec,
            pl.BlockSpec((F,), lambda s: (0,)),
            hbm_spec,
            pl.BlockSpec((D,), lambda s: (0,)),
        ],
        out_specs=pl.BlockSpec((None, D, TM),
                               lambda s: (0, 0, jnp.maximum(s - nt, 0))),
        out_shape=jax.ShapeDtypeStruct((B, D, S), A_x.dtype),
        scratch_shapes=[
            pltpu.VMEM((D, 3 * D), bf16),
            pltpu.VMEM((D, D), bf16),
            pltpu.VMEM((D, F), bf16),
            pltpu.VMEM((D, F), bf16),
            pltpu.VMEM((3 * D, D), bf16),
            pltpu.VMEM((D, S), bf16),
            pltpu.VMEM((D + 16, D), f32),
            pltpu.VMEM((D, D), bf16),
            pltpu.VMEM((2 * H, D), bf16),
            pltpu.VMEM((D, 2 * H), bf16),
            pltpu.VMEM((1, F), f32),
            pltpu.VMEM((D, 128), f32),
            pltpu.SemaphoreType.DMA((4,)),
        ],
        compiler_params=pltpu.CompilerParams(
            dimension_semantics=("arbitrary",),
            vmem_limit_bytes=100 * 1024 * 1024,
        ),
    )(xt, A_wqkv, A_wo, B_w1, B_b1, w2t, B_b2)
    return jnp.transpose(out_t, (0, 2, 1))
```

```python
import functools

import jax
import jax.numpy as jnp
from jax import lax
import jax.experimental.pallas as pl
import jax.experimental.pallas.tpu as pltpu

H = 32
LN_EPS = 1e-5
PHI_EPS = 1e-6
DEN_EPS = 1e-6

TM = 512
TF = 512

NT_DIMS = (((1,), (1,)), ((), ()))


def _ln_t(x):
    m = jnp.mean(x, axis=0, keepdims=True)
    xc = x - m
    v = jnp.mean(xc * xc, axis=0, keepdims=True)
    return xc * lax.rsqrt(v + LN_EPS)


def _phi(t):
    return jnp.where(t > 0, t + 1.0, jnp.exp(t)) + PHI_EPS


def _kv_groups(D, DH):
    groups = []
    for c0 in range(0, D, 128):
        c1 = min(c0 + 128, D)
        r0 = (c0 // DH) * DH
        r1 = ((c1 - 1) // DH + 1) * DH
        groups.append((c0, c1, (r0 // 16) * 16, min(-(-r1 // 16) * 16, D)))
    return groups


def _kernel(x_hbm, wqkv_hbm, wo_hbm, w1_hbm, b1_ref, w2t_hbm, b2_ref, o_ref,
            x_s, wqkv_s, wo_s, w1_s, w2t_s, st_s, wqkvt_s, pqt_s, kv_s, z_s,
            mt_s, zb_s, b1_s, b2_s, sems, *, S, D, F, nt):
    f32 = jnp.float32
    bf16 = jnp.bfloat16
    DH = D // H
    step = pl.program_id(0)
    ka = (D // 128) * 128
    qkv_chunks = [(ka, 2 * D), (2 * D, 3 * D), (0, ka)]

    def copy(src, dst, i):
        return pltpu.make_async_copy(src, dst, sems.at[i])

    def x0_copy():
        return copy(x_hbm.at[0, :, 0:TM], x_s.at[:, 0:TM], 0)

    def xrest_copy():
        return copy(x_hbm.at[0, :, TM:S], x_s.at[:, TM:S], 1)

    def wqkv_copy(i):
        c0, c1 = qkv_chunks[i]
        return copy(wqkv_hbm.at[:, c0:c1], wqkv_s.at[:, c0:c1], 5 + i)

    def stage_rows(val, row0=0):
        ncol = val.shape[1]
        for t, c0 in enumerate(range(0, ncol, 128)):
            c1 = min(c0 + 128, ncol)
            st_s[t, row0:row0 + val.shape[0], 0:c1 - c0] = val[:, c0:c1]

    def permute_staged(dst_ref, ncol, dtype):
        for t, c0 in enumerate(range(0, ncol, 128)):
            c1 = min(c0 + 128, ncol)
            for e in range(DH):
                dst_ref[e * H:(e + 1) * H, c0:c1] = (
                    st_s[t, pl.ds(e, H, stride=DH), 0:c1 - c0].astype(dtype))

    def wt_chunk(i):
        c0, c1 = qkv_chunks[i]
        return jnp.transpose(wqkv_s[:, c0:c1].astype(f32))

    def phase1(col0, first):
        if first:
            x0_copy().start()
            wqkv_copy(0).start()
            kv_s[...] = jnp.zeros(kv_s.shape, f32)
            z_s[...] = jnp.zeros(z_s.shape, f32)
            b1_s[...] = b1_ref[...].astype(f32).reshape(1, F)
            b2row = jnp.broadcast_to(b2_ref[...].astype(f32).reshape(1, D), (128, D))
            b2_s[...] = jnp.transpose(b2row)
            wqkv_copy(0).wait()
            x0_copy().wait()
            wqkv_copy(2).start()
            wt = wt_chunk(0)
            stage_rows(wt[0:D - ka], ka)
            wqkvt_s[D:2 * D, :] = wt[D - ka:].astype(bf16)
        x = x_s[:, pl.ds(col0, TM)].astype(f32)
        ln = _ln_t(x).astype(bf16)
        kt = jnp.dot(wqkvt_s[D:2 * D, :], ln, preferred_element_type=f32)
        pk32 = _phi(kt)
        zpart = pk32[:, 0:128]
        for j in range(1, TM // 128):
            zpart = zpart + pk32[:, j * 128:(j + 1) * 128]
        z_s[...] += zpart
        pk = pk32.astype(bf16)
        if first:
            wqkv_copy(2).wait()
            xrest_copy().start()
            stage_rows(wt_chunk(2), 0)
            permute_staged(wqkvt_s, D, bf16)
        kv_s[...] += lax.dot_general(pk, ln, NT_DIMS, preferred_element_type=f32)
        qt = jnp.dot(wqkvt_s[0:D, :], ln, preferred_element_type=f32)
        pqt_s[:, pl.ds(col0, TM)] = _phi(qt).astype(bf16)

    @pl.when(step == 0)
    def _first():
        phase1(0, True)

    @pl.when(step == 1)
    def _start_weights():
        xrest_copy().wait()
        wqkv_copy(1).start()
        copy(w1_hbm, w1_s, 2).start()
        copy(w2t_hbm, w2t_s, 3).start()
        copy(wo_hbm, wo_s, 4).start()

    @pl.when(jnp.logical_and(step >= 1, step < nt))
    def _phase1():
        phase1(pl.multiple_of(step * TM, TM), False)

    @pl.when(step == nt)
    def _mid():
        copy(wo_hbm, wo_s, 4).wait()
        wqkv_copy(1).wait()
        g = kv_s[...].astype(bf16)
        groups = _kv_groups(D, DH)
        parts = []
        for (c0, c1, r0, r1) in groups:
            r = (lax.broadcasted_iota(jnp.int32, (r1 - r0, c1 - c0), 0) + r0) // DH
            c = (lax.broadcasted_iota(jnp.int32, (r1 - r0, c1 - c0), 1) + c0) // DH
            kvb = jnp.dot(g[r0:r1], wqkv_s[:, 2 * D + c0:2 * D + c1],
                          preferred_element_type=f32)
            blk = jnp.where(r == c, kvb, 0.0).astype(bf16)
            parts.append(jnp.dot(blk, wo_s[c0:c1, :], preferred_element_type=f32))
        bounds = sorted({b for g in groups for b in g[2:]})
        for lo, hi in zip(bounds[:-1], bounds[1:]):
            acc = None
            for (c0, c1, r0, r1), p in zip(groups, parts):
                if r0 <= lo and hi <= r1:
                    piece = p[lo - r0:hi - r0]
                    acc = piece if acc is None else acc + piece
            stage_rows(acc, lo)
        mp = []
        for t, c0 in enumerate(range(0, D, 128)):
            c1 = min(c0 + 128, D)
            mp.append(jnp.concatenate(
                [st_s[t, pl.ds(e, H, stride=DH), 0:c1 - c0] for e in range(DH)], axis=0))
        mt_s[...] = jnp.transpose(jnp.concatenate(mp, axis=1)).astype(bf16)
        z = jnp.sum(z_s[...], axis=1, keepdims=True)
        stage_rows(jnp.broadcast_to(z, z_s.shape))
        permute_staged(zb_s, 128, f32)
        copy(w1_hbm, w1_s, 2).wait()
        copy(w2t_hbm, w2t_s, 3).wait()

    @pl.when(step >= nt)
    def _phase2():
        col0 = pl.multiple_of((step - nt) * TM, TM)
        pq = pqt_s[:, pl.ds(col0, TM)].astype(f32)
        zb = jnp.concatenate([zb_s[...]] * (TM // 128), axis=1)
        den = jnp.sum((pq * zb).reshape(DH, H, TM), axis=0)
        rcp = 1.0 / (den + DEN_EPS)
        pqs = (pq.reshape(DH, H, TM) * rcp[None]).reshape(D, TM).astype(bf16)
        attn = jnp.dot(mt_s[...], pqs, preferred_element_type=f32)
        h = x_s[:, pl.ds(col0, TM)].astype(f32) + attn
        ln2 = jnp.transpose(_ln_t(h)).astype(bf16)
        acc = h + jnp.concatenate([b2_s[...]] * (TM // 128), axis=1)
        for j in range(F // TF):
            a = jnp.dot(ln2, w1_s[:, j * TF:(j + 1) * TF],
                        preferred_element_type=f32)
            a = a + b1_s[:, j * TF:(j + 1) * TF]
            a = jnp.maximum(a, 0.0)
            a = (a * a).astype(bf16)
            acc = acc + lax.dot_general(w2t_s[:, j * TF:(j + 1) * TF], a, NT_DIMS,
                                        preferred_element_type=f32)
        o_ref[...] = acc.astype(o_ref.dtype)


@jax.jit
def pallas_sequential_preLN__linear_attn_block__dense_activation_squared_relu__prompt_kernel(
    A_x: jax.Array,
    A_wqkv: jax.Array,
    A_wo: jax.Array,
    B_x: jax.Array,
    B_w1: jax.Array,
    B_b1: jax.Array,
    B_w2: jax.Array,
    B_b2: jax.Array,
):
    del B_x
    B, S, D = A_x.shape
    F = B_w1.shape[1]
    assert B == 1 and S % TM == 0 and F % TF == 0 and D % H == 0
    nt = S // TM
    assert nt >= 2
    bf16 = jnp.bfloat16
    f32 = jnp.float32

    kern = functools.partial(_kernel, S=S, D=D, F=F, nt=nt)
    hbm_spec = pl.BlockSpec(memory_space=pltpu.HBM)
    xt = jnp.transpose(A_x, (0, 2, 1))
    w2t = jnp.transpose(B_w2, (1, 0))
    out_t = pl.pallas_call(
        kern,
        grid=(2 * nt,),
        in_specs=[
            hbm_spec,
            hbm_spec,
            hbm_spec,
            hbm_spec,
            pl.BlockSpec((F,), lambda s: (0,)),
            hbm_spec,
            pl.BlockSpec((D,), lambda s: (0,)),
        ],
        out_specs=pl.BlockSpec((None, D, TM),
                               lambda s: (0, 0, jnp.maximum(s - nt, 0))),
        out_shape=jax.ShapeDtypeStruct((B, D, S), A_x.dtype),
        scratch_shapes=[
            pltpu.VMEM((D, S), bf16),
            pltpu.VMEM((D, 3 * D), bf16),
            pltpu.VMEM((D, D), bf16),
            pltpu.VMEM((D, F), bf16),
            pltpu.VMEM((D, F), bf16),
            pltpu.VMEM((-(-D // 128), D, 128), f32),
            pltpu.VMEM((2 * D, D), bf16),
            pltpu.VMEM((D, S), bf16),
            pltpu.VMEM((D, D), f32),
            pltpu.VMEM((D, 128), f32),
            pltpu.VMEM((D, D), bf16),
            pltpu.VMEM((D, 128), f32),
            pltpu.VMEM((1, F), f32),
            pltpu.VMEM((D, 128), f32),
            pltpu.SemaphoreType.DMA((8,)),
        ],
        compiler_params=pltpu.CompilerParams(
            dimension_semantics=("arbitrary",),
            vmem_limit_bytes=100 * 1024 * 1024,
        ),
    )(xt, A_wqkv, A_wo, B_w1, B_b1, w2t, B_b2)
    return jnp.transpose(out_t, (0, 2, 1))
```

```python
import functools

import jax
import jax.numpy as jnp
from jax import lax
import jax.experimental.pallas as pl
import jax.experimental.pallas.tpu as pltpu

H = 32
LN_EPS = 1e-5
PHI_EPS = 1e-6
DEN_EPS = 1e-6

TM = 512
TF = 512

NT_DIMS = (((1,), (1,)), ((), ()))


def _ln_t(x):
    m = jnp.mean(x, axis=0, keepdims=True)
    xc = x - m
    v = jnp.mean(xc * xc, axis=0, keepdims=True)
    return xc * lax.rsqrt(v + LN_EPS)


def _phi(t):
    return jnp.where(t > 0, t + 1.0, jnp.exp(t)) + PHI_EPS


def _kv_groups(D, DH):
    groups = []
    for c0 in range(0, D, 128):
        c1 = min(c0 + 128, D)
        r0 = (c0 // DH) * DH
        r1 = ((c1 - 1) // DH + 1) * DH
        groups.append((c0, c1, (r0 // 16) * 16, min(-(-r1 // 16) * 16, D)))
    return groups


def _kernel(x_hbm, wqkv_hbm, wo_hbm, w1_hbm, b1_ref, w2t_hbm, b2_ref, o_ref,
            x_s, wqkv_s, wo_s, w1_s, w2t_s, st_s, wqkt_s, pqt_s, g_s, z_s,
            mt_s, zb_s, b1_s, b2_s, sems, *, S, D, F, nt):
    f32 = jnp.float32
    bf16 = jnp.bfloat16
    DH = D // H
    step = pl.program_id(0)
    ka = (D // 128) * 128
    qkv_chunks = [(ka, 2 * D), (2 * D, 3 * D), (0, ka)]

    def copy(src, dst, i):
        return pltpu.make_async_copy(src, dst, sems.at[i])

    def x0_copy():
        return copy(x_hbm.at[0, :, 0:TM], x_s.at[:, 0:TM], 0)

    def xrest_copy():
        return copy(x_hbm.at[0, :, TM:S], x_s.at[:, TM:S], 1)

    def wqkv_copy(i):
        c0, c1 = qkv_chunks[i]
        return copy(wqkv_hbm.at[:, c0:c1], wqkv_s.at[:, c0:c1], 5 + i)

    def stage_rows(val, row0=0):
        ncol = val.shape[1]
        for t, c0 in enumerate(range(0, ncol, 128)):
            c1 = min(c0 + 128, ncol)
            st_s[t, row0:row0 + val.shape[0], 0:c1 - c0] = val[:, c0:c1]

    def permute_staged(dst_ref, ncol, dtype):
        for t, c0 in enumerate(range(0, ncol, 128)):
            c1 = min(c0 + 128, ncol)
            for e in range(DH):
                dst_ref[e * H:(e + 1) * H, c0:c1] = (
                    st_s[t, pl.ds(e, H, stride=DH), 0:c1 - c0].astype(dtype))

    def wt_chunk(i):
        c0, c1 = qkv_chunks[i]
        return jnp.transpose(wqkv_s[:, c0:c1].astype(f32))

    def pass1(col0, first):
        if first:
            x0_copy().start()
            wqkv_copy(0).start()
            g_s[...] = jnp.zeros(g_s.shape, f32)
            z_s[...] = jnp.zeros(z_s.shape, f32)
            b1_s[...] = b1_ref[...].astype(f32).reshape(1, F)
            b2row = jnp.broadcast_to(b2_ref[...].astype(f32).reshape(1, D), (128, D))
            b2_s[...] = jnp.transpose(b2row)
            wqkv_copy(0).wait()
            x0_copy().wait()
            wqkv_copy(2).start()
            wt = wt_chunk(0)
            stage_rows(wt[0:D - ka], ka)
            wqkt_s[D:2 * D, :] = wt[D - ka:].astype(bf16)
        x = x_s[:, pl.ds(col0, TM)].astype(f32)
        ln = _ln_t(x).astype(bf16)
        kt = jnp.dot(wqkt_s[D:2 * D, :], ln, preferred_element_type=f32)
        pk32 = _phi(kt)
        zpart = pk32[:, 0:128]
        for j in range(1, TM // 128):
            zpart = zpart + pk32[:, j * 128:(j + 1) * 128]
        z_s[...] += zpart
        pk = pk32.astype(bf16)
        if first:
            wqkv_copy(2).wait()
            xrest_copy().start()
            stage_rows(wt_chunk(2), 0)
            permute_staged(wqkt_s, D, bf16)
        g_s[...] += lax.dot_general(pk, ln, NT_DIMS, preferred_element_type=f32)
        qt = jnp.dot(wqkt_s[0:D, :], ln, preferred_element_type=f32)
        pqt_s[:, pl.ds(col0, TM)] = _phi(qt).astype(bf16)

    @pl.when(step == 0)
    def _first():
        pass1(0, True)

    @pl.when(step == 1)
    def _start_weights():
        xrest_copy().wait()
        wqkv_copy(1).start()
        copy(w1_hbm, w1_s, 2).start()
        copy(w2t_hbm, w2t_s, 3).start()
        copy(wo_hbm, wo_s, 4).start()

    @pl.when(jnp.logical_and(step >= 1, step < nt))
    def _pass1():
        pass1(pl.multiple_of(step * TM, TM), False)

    @pl.when(step == nt)
    def _mid():
        copy(wo_hbm, wo_s, 4).wait()
        wqkv_copy(1).wait()
        g = g_s[...].astype(bf16)
        groups = _kv_groups(D, DH)
        parts = []
        for (c0, c1, r0, r1) in groups:
            r = (lax.broadcasted_iota(jnp.int32, (r1 - r0, c1 - c0), 0) + r0) // DH
            c = (lax.broadcasted_iota(jnp.int32, (r1 - r0, c1 - c0), 1) + c0) // DH
            kvb = jnp.dot(g[r0:r1], wqkv_s[:, 2 * D + c0:2 * D + c1],
                          preferred_element_type=f32)
            blk = jnp.where(r == c, kvb, 0.0).astype(bf16)
            parts.append(jnp.dot(blk, wo_s[c0:c1, :], preferred_element_type=f32))
        bounds = sorted({b for grp in groups for b in grp[2:]})
        for lo, hi in zip(bounds[:-1], bounds[1:]):
            acc = None
            for (c0, c1, r0, r1), p in zip(groups, parts):
                if r0 <= lo and hi <= r1:
                    piece = p[lo - r0:hi - r0]
                    acc = piece if acc is None else acc + piece
            stage_rows(acc, lo)
        mp = []
        for t, c0 in enumerate(range(0, D, 128)):
            c1 = min(c0 + 128, D)
            mp.append(jnp.concatenate(
                [st_s[t, pl.ds(e, H, stride=DH), 0:c1 - c0] for e in range(DH)], axis=0))
        mt_s[...] = jnp.transpose(jnp.concatenate(mp, axis=1)).astype(bf16)
        z = jnp.sum(z_s[...], axis=1, keepdims=True)
        stage_rows(jnp.broadcast_to(z, z_s.shape))
        permute_staged(zb_s, 128, f32)
        copy(w1_hbm, w1_s, 2).wait()
        copy(w2t_hbm, w2t_s, 3).wait()

    @pl.when(step >= nt)
    def _pass2():
        col0 = pl.multiple_of((step - nt) * TM, TM)
        pq = pqt_s[:, pl.ds(col0, TM)].astype(f32)
        zb = jnp.concatenate([zb_s[...]] * (TM // 128), axis=1)
        den = jnp.sum((pq * zb).reshape(DH, H, TM), axis=0)
        rcp = 1.0 / (den + DEN_EPS)
        pqs = (pq.reshape(DH, H, TM) * rcp[None]).reshape(D, TM).astype(bf16)
        attn = jnp.dot(mt_s[...], pqs, preferred_element_type=f32)
        h = x_s[:, pl.ds(col0, TM)].astype(f32) + attn
        ln2 = jnp.transpose(_ln_t(h)).astype(bf16)
        acc = h + jnp.concatenate([b2_s[...]] * (TM // 128), axis=1)
        for j in range(F // TF):
            a = jnp.dot(ln2, w1_s[:, j * TF:(j + 1) * TF],
                        preferred_element_type=f32)
            a = a + b1_s[:, j * TF:(j + 1) * TF]
            a = jnp.maximum(a, 0.0)
            a = (a * a).astype(bf16)
            acc = acc + lax.dot_general(w2t_s[:, j * TF:(j + 1) * TF], a, NT_DIMS,
                                        preferred_element_type=f32)
        o_ref[...] = acc.astype(o_ref.dtype)


@jax.jit
def pallas_sequential_preLN__linear_attn_block__dense_activation_squared_relu__prompt_kernel(
    A_x: jax.Array,
    A_wqkv: jax.Array,
    A_wo: jax.Array,
    B_x: jax.Array,
    B_w1: jax.Array,
    B_b1: jax.Array,
    B_w2: jax.Array,
    B_b2: jax.Array,
):
    del B_x
    B, S, D = A_x.shape
    F = B_w1.shape[1]
    assert B == 1 and S % TM == 0 and F % TF == 0 and D % H == 0
    nt = S // TM
    assert nt >= 2
    bf16 = jnp.bfloat16
    f32 = jnp.float32

    kern = functools.partial(_kernel, S=S, D=D, F=F, nt=nt)
    hbm_spec = pl.BlockSpec(memory_space=pltpu.HBM)
    xt = jnp.transpose(A_x, (0, 2, 1))
    w2t = jnp.transpose(B_w2, (1, 0))
    out_t = pl.pallas_call(
        kern,
        grid=(2 * nt,),
        in_specs=[
            hbm_spec,
            hbm_spec,
            hbm_spec,
            hbm_spec,
            pl.BlockSpec((F,), lambda s: (0,)),
            hbm_spec,
            pl.BlockSpec((D,), lambda s: (0,)),
        ],
        out_specs=pl.BlockSpec((None, D, TM),
                               lambda s: (0, 0, jnp.maximum(s - nt, 0))),
        out_shape=jax.ShapeDtypeStruct((B, D, S), A_x.dtype),
        scratch_shapes=[
            pltpu.VMEM((D, S), bf16),
            pltpu.VMEM((D, 3 * D), bf16),
            pltpu.VMEM((D, D), bf16),
            pltpu.VMEM((D, F), bf16),
            pltpu.VMEM((D, F), bf16),
            pltpu.VMEM((-(-D // 128), D, 128), f32),
            pltpu.VMEM((2 * D, D), bf16),
            pltpu.VMEM((D, S), bf16),
            pltpu.VMEM((D, D), f32),
            pltpu.VMEM((D, 128), f32),
            pltpu.VMEM((D, D), bf16),
            pltpu.VMEM((D, 128), f32),
            pltpu.VMEM((1, F), f32),
            pltpu.VMEM((D, 128), f32),
            pltpu.SemaphoreType.DMA((8,)),
        ],
        compiler_params=pltpu.CompilerParams(
            dimension_semantics=("arbitrary",),
            vmem_limit_bytes=100 * 1024 * 1024,
        ),
    )(xt, A_wqkv, A_wo, B_w1, B_b1, w2t, B_b2)
    return jnp.transpose(out_t, (0, 2, 1))
```
